```python
import os as _os
_os.environ.setdefault("JAX_PLATFORMS", "cpu")
import jax
import jax.numpy as jnp

def _softmax(x, axis=-1):
    return jax.nn.softmax(x, axis=axis)
def _gelu(x):
    return jax.nn.gelu(x, approximate=True)
def _silu(x):
    return jax.nn.silu(x)
def _sigmoid(x):
    return jax.nn.sigmoid(x)
def _layernorm(x, axis=-1, eps=1e-5):
    m = jnp.mean(x, axis=axis, keepdims=True)
    v = jnp.var(x, axis=axis, keepdims=True)
    return (x - m) / jnp.sqrt(v + eps)
def _scatter_add(tgt, idx, src, axis=0):
    return tgt.at[idx].add(src)
def _segment_sum(src, seg, n):
    return jax.ops.segment_sum(src, seg, n)
class _Rng:
    def __init__(self, key):
        self._k = key
    def _next(self):
        self._k, sub = jax.random.split(self._k)
        return sub
    def normal(self, shape):
        return jax.random.normal(self._next(), shape, dtype=jnp.bfloat16)
    def randint(self, lo, hi, shape):
        return jax.random.randint(self._next(), shape, lo, hi, dtype=jnp.int32)
    def uniform(self, shape, lo=0.0, hi=1.0):
        return jax.random.uniform(self._next(), shape, jnp.bfloat16, lo, hi)
    def permutation(self, n):
        return jax.random.permutation(self._next(), n)


kernel_name = 'gated_mix__linear_attn_block__swiglu_ffn__prompt'

def setup_inputs():
    _rng = _Rng(jax.random.key(int.from_bytes(__import__("os").urandom(4), "little")))
    _w = (lambda a: (lambda t: t.astype(jnp.bfloat16) if jnp.issubdtype(t.dtype, jnp.floating) else t)(jnp.asarray(a)))
    def _A_setup():
        B, S, D = 1, 2048, 512
        return {
            "x": _w((lambda *s: _rng.normal(s) * 0.05)(B, S, D)),
            "wqkv": _w((lambda *s: _rng.normal(s) * 0.8)(D, 3 * D)),
            "wo": _w((lambda *s: _rng.normal(s) * 0.05)(D, D)),
        }
    _A_in = _A_setup()

    def _B_setup():
        B, S, D, F = 1, 2048, 512, 1792
        return {
            "x": _w((lambda *s: _rng.normal(s) * 0.05)(B, S, D)),
            "w_gate": _w((lambda *s: _rng.normal(s) * 0.1)(D, F)),
            "w_up": _w((lambda *s: _rng.normal(s) * 0.1)(D, F)),
            "w_down": _w((lambda *s: _rng.normal(s) * 0.1)(F, D)),
        }
    _B_in = _B_setup()

    return {
        "A_x": _A_in["x"],
        "A_wqkv": _A_in["wqkv"],
        "A_wo": _A_in["wo"],
        "B_x": _B_in["x"],
        "B_w_gate": _B_in["w_gate"],
        "B_w_up": _B_in["w_up"],
        "B_w_down": _B_in["w_down"],
        "gate_w": _w((lambda *s: _rng.normal(s) * 0.05)(512) * 16.0),
    }

def reference(A_x, A_wqkv, A_wo, B_x, B_w_gate, B_w_up, B_w_down, gate_w):
    def _A_ref(x, wqkv, wo):
        B, S, D = x.shape
        H = 32; Dh = D // H
        qkv = (lambda x, *d: x.transpose(*d))((x @ wqkv).reshape(B, S, 3, H, Dh), 2, 0, 3, 1, 4)
        q, k, v = qkv[0], qkv[1], qkv[2]
        phi = lambda t: jnp.where(t > 0, t + 1, jnp.exp(t)) + 1e-6
        pq, pk = phi(q), phi(k)
        kv = jnp.einsum("bhsd,bhse->bhde", pk, v)
        z = jnp.einsum("bhsd->bhd", pk)
        num = jnp.einsum("bhqd,bhde->bhqe", pq, kv)
        den = jnp.einsum("bhqd,bhd->bhq", pq, z)[..., None] + 1e-6
        o = num / den
        return (lambda x, *d: x.transpose(*d))(o, 0, 2, 1, 3).reshape(B, S, D) @ wo

    def _B_ref(x, w_gate, w_up, w_down):
        g = _silu(x @ w_gate)
        u = x @ w_up
        return (g * u) @ w_down

    x = A_x
    g = _sigmoid((x * gate_w).sum(-1, keepdims=True))
    a = _A_ref(x, A_wqkv, A_wo)
    b = _B_ref(x, B_w_gate, B_w_up, B_w_down)
    return g * a + (1 - g) * b
```

```python
import functools
import jax, jax.numpy as jnp
from jax import lax
import jax.experimental.pallas as pl
import jax.experimental.pallas.tpu as pltpu

S, D, F, H, DH = 2048, 512, 1792, 32, 16
T = 128
f32, bf16, u32 = jnp.float32, jnp.bfloat16, jnp.uint32
lazy = functools.cache


def nn(a, b):
    return jnp.dot(a, b, preferred_element_type=f32)


def nt(a, b):
    return lax.dot_general(a, b, (((1,), (1,)), ((), ())), preferred_element_type=f32)


LHS = [((0, 1), (3, 1)), ((2, 1), (3, 1)), ((0, 1),), ((3, 1),), ((0, 1), (1, 1)), ((2, 1), (0, -1)), ((1, 1), (3, -1))]
RHS = [((0, 1), (3, 1)), ((0, 1),), ((1, 1), (3, -1)), ((2, 1), (0, -1)), ((3, 1),), ((0, 1), (1, 1)), ((2, 1), (3, 1))]
OUT = [((0, 1), (3, 1), (4, -1), (6, 1)), ((2, 1), (4, 1)), ((1, 1), (3, 1)), ((0, 1), (1, -1), (2, 1), (5, 1))]
RHS_FROM_LHS = [0, 2, 6, 5, 3, 4, 1]


def ssum(terms):
    if terms[0][1] < 0:
        terms = [terms[1], terms[0], *terms[2:]]
    v = terms[0][0]
    for w, sg in terms[1:]:
        v = v + w if sg > 0 else v - w
    return v


def dec(m, k, order, init=None):
    terms = [(m(i), sg) for i, sg in sorted(OUT[k], key=lambda t: order.index(t[0]))]
    return ssum(terms if init is None else [(init, 1)] + terms)


def cat(vs, axis=0):
    return vs[0] if len(vs) == 1 else jnp.concatenate(vs, axis=axis)


def tree(vs):
    while len(vs) > 1:
        vs = [vs[i] + vs[i + 1] if i + 1 < len(vs) else vs[i] for i in range(0, len(vs), 2)]
    return vs[0]


def enc1(spec, blk):
    blk = lazy(blk)
    op = lazy(lambda q: ssum([(blk(b // 2, b % 2), sb) for b, sb in spec[q]]))
    res = lazy(lambda q: op(q).astype(bf16))
    def hints(st=16):
        for r0 in range(0, blk(0, 0).shape[0], st):
            for q in ((5, 6) if spec is RHS else (4, 1)):
                yield op(q)[r0:r0 + st]
    res.hints = hints
    return res


def enc2(spec, blk, flat=0, touch=None):
    blk = lazy(blk)
    at = lambda a, b: blk(2 * (a // 2) + b // 2, 2 * (a % 2) + b % 2)
    t = lazy(lambda p, b: ssum([(at(a, b), sa) for a, sa in spec[p]]))
    @lazy
    def op(p, q):
        if flat:
            terms = [(at(a, b), sa * sb) for a, sa in spec[p] for b, sb in spec[q]]
            if len(terms) == 4:
                terms = [terms[0], terms[3], terms[1], terms[2]]
            v = ssum(terms)
            if flat == 2 and len(terms) == 1:
                for b in (1, 2):
                    v = touch(at(p - 1, b), v)
            return v
        return ssum([(t(p, b), sb) for b, sb in spec[q]])
    res = lazy(lambda p, q: op(p, q).astype(bf16))
    def hints(st=16):
        for r0 in range(0, blk(0, 0).shape[0], st):
            for p in range(7):
                for q in ((5, 6) if spec is RHS else (4, 1)):
                    yield op(p, q)[r0:r0 + st]
    res.hints = hints
    return res


def build(R=128, qord=(0, 5, 6, 1, 2, 3, 4), pord=(3, 1, 2, 4, 0, 5, 6), flags=None, lp=1, prof=0,
          fh=2, fx=0, fw=0, fp=2, dg=1, du=1, pre=1, sched=0, pdown=None, qdown=(2, 3, 0, 4, 6, 1, 5), qlast=(2, 3, 4, 1, 0, 6, 5),
          pins=(6, 4), slots=((3, 4), (1, 6), (2, 4), (4, 6), (0, 4), (5, 6)), half=1, sp=1.8, wt_=(1, 1.2, 0.5, 0, 2), rcp=0, q0=None):
    NS = S // (4 * R)
    RB = 4 * R
    flags = dict(flags or {})
    if lp:
        flags['XLA_TPU_FORCE_LP_LLO_SCHEDULER'] = True
    pdown = pdown or pord

    def phi(t):
        return (jnp.maximum(t, 0.0) + 1e-6) + jnp.exp(jnp.minimum(t, 0.0))

    def kern(x_hbm, wqkv_hbm, wo_hbm, wg_hbm, wu_hbm, wd_hbm, gw_hbm, o_hbm,
             x_v, wqkv_v, wo_v, wg_v, wu_v, wd_v, gw_v, o_v, tr, tr2, sem):
        def cols(c0, n):
            return lambda ref: ref.at[:, pl.ds(c0, n)]
        def rows(r0, n):
            return lambda ref: ref.at[pl.ds(r0, n)]
        whole = lambda ref: ref
        def fetch(k, *items):
            cps = [pltpu.make_async_copy(view(src), view(dst), sem.at[k]) for src, dst, view in items]
            for c in cps:
                c.start()
            return cps
        scope = [None, 0]
        def mark(name):
            if not prof:
                return
            if scope[0]:
                scope[0].__exit__(None, None, None)
            scope[1] += 1
            scope[0] = name and jax.named_scope(f"z{scope[1]:02d}_{name}")
            if name:
                scope[0].__enter__()
        def wait(cps):
            mark("wait")
            for c in cps:
                c.wait()
            mark("run")

        @lazy
        def never(shape):
            i = lax.broadcasted_iota(jnp.int32, shape, 1)
            return (i * (i + 1)) & 1 == 1
        touch = lambda v, r: jnp.where(never(r.shape), v, r)
        todo = []
        credit = [0.0]
        def early(gen, n, sets):
            todo.append((gen, n / (len(slots) * sets)))
        xw = lazy(lambda s, p, q: pltpu.bitcast(xc[s](p, q), u32))
        def carry(r, weight):
            vs = []
            if todo:
                credit[0] += todo[0][1] * weight
            while weight and credit[0] >= 1 - 1e-9 and todo:
                v = next(todo[0][0], None)
                if v is None:
                    todo.pop(0)
                else:
                    vs.append(lax.bitcast_convert_type(v, u32)); credit[0] -= 1
            if vs:
                parts = [r[k:k + 16] for k in range(0, r.shape[0], 16)]
                for k, v in enumerate(vs):
                    j = k * len(parts) // len(vs)
                    parts[j] = touch(v, parts[j])
                r = cat(parts)
            return pltpu.bitcast(r, bf16)
        def xop(s, p, q, weight):
            return carry(xw(s, p, q), weight) if (p, q) in slots else xc[s](p, q)

        def direct(w, c0, s, perm, scale):
            out = {}
            for n in range(4):
                xs = [x_v[pl.ds(s * RB, RB), pl.ds(c * T, T)] for c in range(4)]
                xs[0] = carry(pltpu.bitcast(xs[0], u32), len(slots) / 4)
                out[n] = scale(tree([nn(xs[c], w[pl.ds(c * T, T), pl.ds(c0 + (n ^ perm) * T, T)]) for c in range(4)]))
            return lambda r, n: out[n][r * R:(r + 1) * R]

        def group(prod, qs):
            pr = {q: prod(q) for q in qs}
            return [dec(pr.get, k, qs) for k in range(4)]

        def matmul2(prod, ps=pord, qs=qord):
            m = {p: group(functools.partial(prod, p), qs) for p in ps}
            return lazy(lambda r, n, : dec(lambda p: m[p][2 * (r % 2) + n % 2], 2 * (r // 2) + n // 2, ps))

        def ld(ref, r, c, n=T):
            return ref[pl.ds(r, n), pl.ds(c, T)].astype(f32)

        gs = (lambda v: 0.5 * v) if half else (lambda v: v)
        ws = {}
        for u in range(3):
            ws["g", u] = enc2(RHS, lambda r, n, u=u: gs(ld(wg_v, r * T, 512 * u + n * T)), fw)
            ws["u", u] = enc2(RHS, lambda r, n, u=u: ld(wu_v, r * T, 512 * u + (n ^ 3) * T), fw)

        xb = lazy(lambda s, r, c: ld(x_v, s * RB + r * R, c * T, R))
        xc = [enc2(LHS, functools.partial(xb, s), fx) for s in range(NS)]

        @lazy
        def og(s, r):
            gw = gw_v[...].astype(f32).reshape(1, D)
            t = tree([xb(s, r, c) * gw[:, c * T:(c + 1) * T] for c in range(4)])
            return jnp.broadcast_to(0.5 - 0.5 * jnp.tanh(0.5 * jnp.sum(t, axis=-1, keepdims=True)), (R, T))

        def silu(g):
            hh = g if half else 0.5 * g
            return hh * jnp.tanh(hh) + hh
        gate_mm = lazy(lambda u, s: direct(wg_v, 0, s, 0, gs) if (u, s) == (0, 0) and dg else matmul2(lambda p, q: nn(xop(s, p, q, wt_[0]), ws["g", u](p, q)), qs=q0 if (q0 and u == 0) else qord))
        up_mm = lazy(lambda u, s: direct(wu_v, 0, s, 3, lambda v: v) if (u, s) == (0, 0) and du else matmul2(lambda p, q: nn(xop(s, p, q, wt_[1]), ws["u", u](p, q))))
        sg = lazy(lambda u, s, r, n: silu(gate_mm(u, s)(r, n)))
        hid = lazy(lambda u, s, r, n: (sg(u, s, r, n) * up_mm(u, s)(r, n ^ 3)) * og(s, r))
        def force(f, *a):
            for r in range(4):
                for n in range(4):
                    f(*a, r, n)

        def prm(ref, c, n):
            return cat([ref[c, pl.ds(4 * n + d, H, stride=DH), :] for d in range(4)])

        wT = lazy(lambda c, n: ld(wqkv_v, c * T, n * T).T)
        wk = enc2(RHS, lambda c, n: wT(c, 4 + n), fw)
        k_mm = lazy(lambda s: matmul2(lambda p, q: nt(wk(p, q), xop(s, p, q, wt_[2]))))
        pk = lazy(lambda s, n, r: phi(k_mm(s)(r, n)))
        pc = [enc2(LHS, functools.partial(pk, s), fp, touch) for s in range(NS)]
        G = lazy(lambda: matmul2(lambda p, q: tree([nn(pc[s](p, q), xop(s, RHS_FROM_LHS[p], RHS_FROM_LHS[q], 0)) for s in range(NS)]), pdown, qdown))

        @lazy
        def kv():
            ri = lax.broadcasted_iota(jnp.int32, (T, T), 0) // DH
            ci = lax.broadcasted_iota(jnp.int32, (T, T), 1) // DH
            vs = [nn(cat([G()(n, c) for c in range(4)], 1).astype(bf16), wqkv_v[:, pl.ds(2 * D + n * T, T)]) for n in range(4)]
            return [jnp.where(ri == ci, v, 0.0).astype(bf16) for v in vs]

        def m_step():
            for n in range(4):
                mm = nn(kv()[n], wo_v[pl.ds(n * T, T), :])
                for c in range(4):
                    tr[c, pl.ds(n * T, T), :] = mm[:, c * T:(c + 1) * T]

        @lazy
        def zp():
            for n in range(4):
                zs = ssum([((pk(s, n, 0) + pk(s, n, 1)) + (pk(s, n, 2) + pk(s, n, 3)), 1) for s in range(NS)])
                tr[4, pl.ds(n * T, T), :] = tree([zs[:, t * T:(t + 1) * T] for t in range(R // T)])
            return [jnp.sum(prm(tr, 4, n).T, axis=0, keepdims=True) for n in range(4)]

        @lazy
        def wq_col(c):
            tr2[c] = cat([wT(c, n) for n in range(4)])
        wq = enc2(RHS, lambda c, n: wq_col(c) or prm(tr2, c, n), fw)
        q_mm = lazy(lambda s: matmul2(lambda p, q: nt(xop(s, p, q, wt_[3]), wq(p, q))))

        @lazy
        def attn(s, r):
            pq = [phi(q_mm(s)(r, n)) for n in range(4)]
            den = tree([pq[n] * zp()[n] for n in range(4)])
            den = den + pltpu.roll(den, 64, 1)
            den = den + pltpu.roll(den, 32, 1)
            sc = (1.0 - og(s, r)) / (den + 1e-6)
            return [v * sc for v in pq]

        c0 = 1536
        wt = [[enc1(RHS, lambda i, j, J=J: gs(ld(wg_v, (2 * J + i) * T, c0 + j * T))) for J in range(2)],
              [enc1(RHS, lambda i, j, J=J: ld(wu_v, (2 * J + i) * T, c0 + (j ^ 1) * T)) for J in range(2)]]
        dt = [enc1(RHS, lambda i, j, N=N: ld(wd_v, c0 + i * T, (2 * N + j) * T)) for N in range(2)]
        @lazy
        def tail(s, I):
            xt = enc1(LHS, lambda i, j: ld(x_v, s * RB + (2 * I + i) * R, (2 * (1 - I) + j) * T, R))
            g, v = [group(lambda q: nn(xop(s, 2 + I, q, wt_[4]), w[I](q)) + nn(xt(q), w[1 - I](q)), qord) for w in wt]
            return enc1(LHS, lambda i, j: (silu(g[2 * i + j]) * v[2 * i + (j ^ 1)]) * og(s, 2 * I + i))

        dc = [enc2(RHS, lambda r, n, u=u: ld(wd_v, 512 * u + r * T, n * T), fw) for u in range(3)] + [enc2(RHS, lambda n, c: prm(tr, c, n), fw)]
        outs = []
        def down(s):
            hc = [enc2(LHS, functools.partial(hid, u, s), fh, touch) for u in range(3)] + [enc2(LHS, lambda r, n: attn(s, r)[n], fh, touch)]
            c1 = [group(lambda q: nn(tail(s, I)(q), dt[N](q)), qord) for I in range(2) for N in range(2)]
            last = s == NS - 1
            m = {}
            for p in pdown:
                fin = last and p == pdown[-1]
                m[p] = group(lambda q: tree([nn(hc[u](p, q), dc[u](p, q)) for u in range(4)]), qlast if fin else qdown)
                for K in range(4):
                    if p in dict(OUT[K]) and all(i in m for i, _ in OUT[K]):
                        for k in (1, 2, 0, 3):
                            r, n = 2 * (K // 2) + k // 2, 2 * (K % 2) + k % 2
                            at = lambda ref, w=T: ref.at[pl.ds(s * RB + r * R, R), pl.ds(n * T, w)]
                            at(o_v)[...] = dec(lambda i: m[i][k], K, pdown, c1[K][k]).astype(bf16)
                            if fin:
                                outs.extend(fetch(5, (o_v, o_hbm, at)))
                        if last and not fin:
                            outs.extend(fetch(5, (o_v, o_hbm, lambda ref: ref.at[pl.ds(s * RB + (K // 2) * 2 * R, 2 * R), pl.ds((K % 2) * 2 * T, 2 * T)])))
            if not last:
                outs.extend(fetch(5, (o_v, o_hbm, rows(s * RB, RB))))

        def all49(o):
            for p in range(7):
                for q in range(7):
                    o(p, q)
        def tposes(n0):
            for c in range(4):
                for n in range(4):
                    yield wT(c, n0 + n)[T - 16:]
        a = fetch(0, (wg_hbm, wg_v, cols(0, 512)))
        b = fetch(1, (x_hbm, x_v, rows(0, RB)), (gw_hbm, gw_v, whole))
        c = fetch(2, (wu_hbm, wu_v, cols(0, 512)), (x_hbm, x_v, rows(RB, RB)))
        d = fetch(3, (x_hbm, x_v, rows(2 * RB, S - 2 * RB)), (wg_hbm, wg_v, cols(512, 512)), (wu_hbm, wu_v, cols(512, 512)))
        e = fetch(4, (wqkv_hbm, wqkv_v, whole), (wg_hbm, wg_v, cols(1024, F - 1024)), (wu_hbm, wu_v, cols(1024, F - 1024)),
                  (wo_hbm, wo_v, whole), (wd_hbm, wd_v, whole))
        nx = 14 * R // 16
        def gates(s):
            for r in range(4):
                og(s, r)
        wait(a)
        if pre:
            all49(ws["g", 0])
        wait(b)
        if not pre:
            early(ws["g", 0].hints(), 112, 0.5)
        if dg:
            early(xc[0].hints(), nx, 1 if pre else 0.5)
        force(sg, 0, 0)
        all49(xc[0]); all49(ws["g", 0]); gates(0)
        wait(c)
        early(xc[1].hints(), nx, 0.65); early(ws["u", 0].hints(), 112, 1.0)
        force(hid, 0, 0)
        force(sg, 0, 1)
        all49(ws["u", 0]); gates(1)
        wait(d)
        early(xc[2].hints(), nx, 1); early(xc[3].hints(), nx, 2)
        early(ws["g", 1].hints(), 112, 1.9); early(ws["u", 1].hints(), 112, 2)
        force(hid, 0, 1); force(hid, 0, 2); force(hid, 0, 3)
        force(sg, 1, 0); force(sg, 1, 1)
        all49(ws["u", 1])
        wait(e)
        early(ws["g", 2].hints(), 112, sp); early(tposes(4), 16, 0.5 * sp); early(wk.hints(), 112, sp)
        early(ws["u", 2].hints(), 112, sp)
        early(tposes(0), 16, 0.5 * sp); early(wq.hints(), 112, sp)
        for o in (*wt[0], *wt[1], *dt):
            early(o.hints(), 16, 0.15 * sp)
        for u in range(3):
            early(dc[u].hints(), 112, sp)
        for s in range(NS):
            force(hid, 1, s)
        for s in range(NS):
            k_mm(s)
        gate_mm(2, 0); G(); up_mm(2, 0); kv(); gate_mm(2, 1); m_step(); up_mm(2, 1)
        early(dc[3].hints(), 112, sp)
        if sched == 0:
            for s in range(2, NS):
                force(hid, 2, s)
            for s in range(NS):
                q_mm(s); tail(s, 0); tail(s, 1)
        else:
            for s in range(NS):
                q_mm(s); tail(s, 0); tail(s, 1)
            for s in range(2, NS):
                force(hid, 2, s)
        for s in range(NS):
            down(s)
        wait(outs)
        mark(None)

    def fn(A_x, A_wqkv, A_wo, B_x, B_w_gate, B_w_up, B_w_down, gate_w):
        any_ = pl.BlockSpec(memory_space=pl.ANY)
        out = pl.pallas_call(
            kern,
            in_specs=[any_] * 7,
            out_specs=any_,
            out_shape=jax.ShapeDtypeStruct((S, D), bf16),
            scratch_shapes=[
                pltpu.VMEM((S, D), bf16), pltpu.VMEM((D, 3 * D), bf16), pltpu.VMEM((D, D), bf16),
                pltpu.VMEM((D, F), bf16), pltpu.VMEM((D, F), bf16), pltpu.VMEM((F, D), bf16), pltpu.VMEM((D,), bf16),
                pltpu.VMEM((S, D), bf16),
                pltpu.VMEM((5, D, T), f32), pltpu.VMEM((4, D, T), f32),
                pltpu.SemaphoreType.DMA((6,)),
            ],
            compiler_params=pltpu.CompilerParams(vmem_limit_bytes=124 * 2**20, flags=flags),
            name="v7k",
        )(A_x.reshape(S, D), A_wqkv, A_wo, B_w_gate, B_w_up, B_w_down, gate_w)
        return out.reshape(1, S, D)
    return fn


@jax.jit
def pallas_gated_mix__linear_attn_block__swiglu_ffn__prompt_kernel(A_x, A_wqkv, A_wo, B_x, B_w_gate, B_w_up, B_w_down, gate_w):
    return build()(A_x, A_wqkv, A_wo, B_x, B_w_gate, B_w_up, B_w_down, gate_w)
```

```python
import functools

import jax
import jax.numpy as jnp
from jax import lax
import jax.experimental.pallas as pl
import jax.experimental.pallas.tpu as pltpu

S, D, F, DH = 2048, 512, 1792, 16
T = 128
NS = S // D
FT = 3 * D
STRIP = 16
f32, bf16, u32 = jnp.float32, jnp.bfloat16, jnp.uint32
lazy = functools.cache

LHS = [((0, 1), (3, 1)), ((2, 1), (3, 1)), ((0, 1),), ((3, 1),),
       ((0, 1), (1, 1)), ((2, 1), (0, -1)), ((1, 1), (3, -1))]
RHS = [((0, 1), (3, 1)), ((0, 1),), ((1, 1), (3, -1)), ((2, 1), (0, -1)),
       ((3, 1),), ((0, 1), (1, 1)), ((2, 1), (3, 1))]
OUT = [((0, 1), (3, 1), (4, -1), (6, 1)), ((2, 1), (4, 1)),
       ((1, 1), (3, 1)), ((0, 1), (1, -1), (2, 1), (5, 1))]
RHS_AS_LHS = [LHS.index(terms) for terms in RHS]
OUTER_ORDER = (1, 3, 2, 4, 0, 5, 6)
INNER_ORDER = (4, 2, 3, 6, 0, 1, 5)
PACE = dict(zip(OUTER_ORDER, (1, 0.25, 1, 0.25, 1, 0.25, 0)))


def _nn(a, b):
    return jnp.dot(a, b, preferred_element_type=f32)


def _nt(a, b):
    return lax.dot_general(a, b, (((1,), (1,)), ((), ())), preferred_element_type=f32)


def _signed_sum(terms):
    if terms[0][1] < 0:
        terms = [terms[1], terms[0], *terms[2:]]
    total = terms[0][0]
    for v, sign in terms[1:]:
        total = total + v if sign > 0 else total - v
    return total


def _sum4(v):
    return (v[0] + v[1]) + (v[2] + v[3])


def _tile(outer, inner):
    return 2 * (outer // 2) + inner // 2, 2 * (outer % 2) + inner % 2


def _combine(product, quadrant, order, init=None):
    terms = sorted(OUT[quadrant], key=lambda t: order.index(t[0]))
    terms = [(product(i), sign) for i, sign in terms]
    return _signed_sum(terms if init is None else [(init, 1)] + terms)


def _operands1(spec, tile):
    tile = lazy(tile)
    return lazy(lambda q: _signed_sum(
        [(tile(b // 2, b % 2), sign) for b, sign in spec[q]]).astype(bf16))


def _left_operands2(tile):
    tile = lazy(tile)

    @lazy
    def operand(p, q):
        t = [(tile(*_tile(a, b)), sa * sb) for a, sa in LHS[p] for b, sb in LHS[q]]
        return _signed_sum([t[0], t[3], t[1], t[2]] if len(t) == 4 else t)
    return operand


def _phi(t):
    return (jnp.maximum(t, 0.0) + 1e-6) + jnp.exp(jnp.minimum(t, 0.0))


def _silu_of_double(h):
    return h * jnp.tanh(h) + h


def _kernel(x_hbm, wqkv_hbm, wo_hbm, wg_hbm, wu_hbm, wd_hbm, gw_hbm, o_hbm,
            x_v, wqkv_v, wo_v, wg_v, wu_v, wd_v, gw_v, o_v, sems):

    def start(sem, *items):
        copies = [pltpu.make_async_copy(view(src), view(dst), sems.at[sem])
                  for src, dst, view in items]
        for c in copies:
            c.start()
        return copies

    def wait(copies):
        assert not queue
        for c in copies:
            c.wait()

    def cols(c0, n):
        return lambda ref: ref.at[:, pl.ds(c0, n)]

    def rows(r0, n):
        return lambda ref: ref.at[pl.ds(r0, n)]

    def whole(ref):
        return ref

    def load(ref, r0, c0):
        return ref[pl.ds(r0, T), pl.ds(c0, T)].astype(f32)

    lane = lazy(lambda n: lax.broadcasted_iota(jnp.int32, (n, T), 1))

    queue, state = [], {"credit": 0.0, "count": 0}
    never = lazy(lambda n: (lane(n) * (lane(n) + 1)) & 1 == 1)

    def advance(amount, result):
        state["credit"] += amount
        state["count"] += 1
        due = []
        while queue and state["credit"] >= queue[0][1] - 1e-6:
            step, cost = queue.pop(0)
            state["credit"] -= cost
            due.append(step)
        if not queue:
            state["credit"] = 0.0
        strips = result.shape[0] // STRIP
        shift = 3 * state["count"] if result.shape[0] == T else 0
        for i, step in enumerate(due):
            def after(v, r0=(i * strips // len(due) + shift) % strips * STRIP):
                n = v.shape[0]
                other = result[r0:r0 + n] if n == STRIP else result[:n]
                return jnp.where(never(n), lax.bitcast_convert_type(other, v.dtype), v)
            step(after)
        return result

    def prepare(spec, tile, cost, outer=range(7)):
        tile, parts, operands = lazy(tile), {}, {}

        def step(r0, p, after):
            t = [_signed_sum([(tile(*_tile(a, b))[r0:r0 + STRIP], sign) for a, sign in spec[p]])
                 for b in range(4)]
            t[0], t[3] = after(t[0]), after(t[3])
            for q in range(7):
                parts.setdefault((p, q), []).append(
                    _signed_sum([(t[b], sign) for b, sign in spec[q]]))
                if r0 + STRIP == T:
                    operands[p, q] = jnp.concatenate(parts[p, q]).astype(bf16)

        for r0 in range(0, T, STRIP):
            for p in outer:
                if cost:
                    queue.append(
                        (functools.partial(step, r0, p), cost * STRIP / (len(outer) * T)))
                else:
                    step(r0, p, lambda v: v)
        return operands

    def strassen1(product, amount=0):
        results = {q: advance(amount, product(q)) for q in INNER_ORDER}
        return [_combine(results.get, k, INNER_ORDER) for k in range(4)]

    mm = {}

    def strassen2(name, product, amount=1, pace=PACE, left=0, hook=None):
        m, remaining = {}, [49]
        mm[name] = lazy(lambda r, n: _combine(
            lambda p: m[p][2 * (r % 2) + n % 2], 2 * (r // 2) + n // 2, OUTER_ORDER))

        def issue(p, q):
            if remaining[0] == left:
                hook()
            remaining[0] -= 1
            return product(p, q)

        for p in OUTER_ORDER:
            m[p] = strassen1(functools.partial(issue, p),
                             amount * pace[p] / (7 * sum(pace.values())))

    xs, ws = {}, {}

    def project(w, s, **kw):
        strassen2((w, s), lambda p, q: _nn(xs[s][p, q], ws[w][p, q]), **kw)

    def every_tile(f, *args):
        for r in range(4):
            for n in range(4):
                f(*args, r, n)

    x_tile = lazy(lambda s, r, c: load(x_v, s * D + r * T, c * T))

    @lazy
    def ffn_gate(s, r):
        gw = gw_v[...].astype(f32).reshape(1, D)
        t = _sum4([x_tile(s, r, c) * gw[:, c * T:(c + 1) * T] for c in range(4)])
        t = jnp.sum(t, axis=-1, keepdims=True)
        return jnp.broadcast_to(0.5 - 0.5 * jnp.tanh(0.5 * t), (T, T))

    def prepare_x(s, cost):
        xs[s] = prepare(LHS, functools.partial(x_tile, s), cost)
        for r in range(4):
            ffn_gate(s, r)

    def gate_tile(u):
        return lambda c, n: 0.5 * load(wg_v, c * T, u * D + n * T)

    def prepare_gate(u, cost):
        ws["gate", u] = prepare(RHS, gate_tile(u), cost)

    def prepare_up(u, cost):
        ws["up", u] = prepare(RHS, lambda c, n: load(wu_v, c * T, u * D + (3 - n) * T), cost)

    act = lazy(lambda u, s, r, n: _silu_of_double(mm[("gate", u), s](r, n)))
    hidden = lazy(lambda u, s, r, n:
                  (act(u, s, r, n) * mm[("up", u), s](r, 3 - n)) * ffn_gate(s, r))

    first = {}
    mm[("gate", 0), 0] = lambda r, n: first[r, n]

    def first_gate(r0, shares):
        for n, amount in shares.items():
            v = advance(amount, _nn(x_v[pl.ds(r0 * T, 2 * T), :], wg_v[:, pl.ds(n * T, T)]))
            for i in range(2):
                first[r0 + i, n] = 0.5 * v[i * T:(i + 1) * T]
                act(0, 0, r0 + i, n)

    low = lazy(lambda: lane(T) < T // 2)

    def prepare_tail(cost):
        def tile(c, n):
            g = 0.5 * load(wg_v, c * T, FT + (n // 2) * T)
            v = load(wu_v, c * T, FT + (n // 2) * T)
            if n % 2:
                return pltpu.roll(jnp.where(low(), v, g), T // 2, 1)
            return jnp.where(low(), g, v)
        ws["tail"] = prepare(RHS, tile, cost)

    @lazy
    def hidden_tail(s, r, j):
        a = mm["tail", s](r, 2 * j)
        b = pltpu.roll(mm["tail", s](r, 2 * j + 1), T // 2, 1)
        return (_silu_of_double(jnp.where(low(), a, b)) * jnp.where(low(), b, a)) * ffn_gate(s, r)

    def by_dim(r0, n, c0, after):
        words = after(pltpu.bitcast(wqkv_v[pl.ds(r0, n), pl.ds(c0, T)], u32))
        return jnp.take_along_axis(words, (lane(n // 2) % 8) * DH + lane(n // 2) // 8, axis=1)

    def regroup(tiles, t):
        return jnp.concatenate([v[8 * d:8 * d + 8] for d in range(4 * t, 4 * t + 4) for v in tiles])

    def prepare_k(cost):
        wt = {}

        def transpose(c, n, after):
            wt[c, n] = pltpu.bitcast(by_dim(c * T, T, D + n * T, after), bf16).astype(f32).T
        queue.extend((functools.partial(transpose, c, n), cost / 48)
                     for c in range(4) for n in range(4))
        ws["k"] = prepare(RHS, lambda c, n: wt[c, n], cost * 2 / 3)

    def prepare_q(cost):
        wt, w = {}, {}

        def there(c, n, after):
            wt[c, n] = by_dim(2 * c * T, 2 * T, n * T, after).T

        def back(c, t, after):
            w[c, t] = pltpu.bitcast(after(regroup([wt[c, n] for n in range(4)], t)).T, bf16)
        queue.extend((functools.partial(f, c, n), cost / 48)
                     for f in (there, back) for c in range(2) for n in range(4))
        ws["q"] = prepare(
            RHS, lambda c, t: w[c // 2, t][(c % 2) * T:(c % 2 + 1) * T].astype(f32), cost * 2 / 3)

    phi_kt = lazy(lambda s, n, r: _phi(mm["k", s](r, n)))
    ks = [_left_operands2(functools.partial(phi_kt, s)) for s in range(NS)]

    @lazy
    def kv():
        same_head = lax.broadcasted_iota(jnp.int32, (T, T), 0) % 8 == lane(T) // DH
        out = []
        for n in range(4):
            ktx = jnp.concatenate([mm["ktx"](n, c) for c in range(4)], axis=1).astype(bf16)
            v = _nn(ktx, wqkv_v[:, pl.ds(2 * D + n * T, T)])
            out.append(jnp.where(same_head, v, 0.0).astype(bf16))
        return out

    kv_wo = lazy(lambda: [_nn(kv()[n], wo_v[pl.ds(n * T, T), :]) for n in range(4)])

    @lazy
    def z():
        sums = [_sum4([ks[s]((4, 1)[n // 2], (4, 1)[n % 2]) for s in range(NS)])
                for n in range(4)]
        return [jnp.sum(regroup(sums, t).T, axis=0, keepdims=True) for t in range(4)]

    @lazy
    def attention(s, r):
        phi_q = [_phi(mm["q", s](r, t)) for t in range(4)]
        den = _sum4([phi_q[t] * z()[t] for t in range(4)])
        den = den + pltpu.roll(den, 64, 1)
        den = den + pltpu.roll(den, 32, 1)
        return phi_q, (1.0 - ffn_gate(s, r)) * pltpu.reciprocal(den + 1e-6, full_range=False)

    stores = []
    down_tail = [_operands1(RHS, lambda i, j, n=n: load(wd_v, FT + i * T, (2 * n + j) * T))
                 for n in range(2)]

    def output(s, down):
        def store(r0, c0, n):
            view = lambda ref: ref.at[pl.ds(s * D + r0 * T, n * T), pl.ds(c0 * T, n * T)]
            stores.extend(start(len(loads), (o_v, o_hbm, view)))

        hs = [_left_operands2(functools.partial(hidden, u, s)) for u in range(3)]
        hs.append(_left_operands2(lambda r, t: attention(s, r)[0][t] * attention(s, r)[1]))
        ht = [_operands1(LHS, lambda i, j, h=h: hidden_tail(s, 2 * h + i, j)) for h in range(2)]
        tail = [strassen1(lambda q: _nn(ht[k // 2](q), down_tail[k % 2](q))) for k in range(4)]
        m = {}
        for p in OUTER_ORDER:
            m[p] = strassen1(lambda q: _sum4(
                [_nn(hs[u](p, q).astype(bf16), down[u][p, q]) for u in range(4)]))
            for outer in range(4):
                needs = dict(OUT[outer])
                if p not in needs or any(i not in m for i in needs):
                    continue
                for inner in (1, 0, 2, 3):
                    r, n = _tile(outer, inner)
                    v = _combine(lambda i: m[i][inner], outer, OUTER_ORDER, tail[outer][inner])
                    o_v[pl.ds(s * D + r * T, T), pl.ds(n * T, T)] = v.astype(bf16)
                    if s == NS - 1 and len(m) == 7:
                        store(r, n, 1)
                if s == NS - 1 and len(m) < 7:
                    store(*_tile(outer, 0), 2)
        if s < NS - 1:
            store(0, 0, 4)

    loads = [start(i, *items) for i, items in enumerate([
        [(x_hbm, x_v, rows(0, 2 * T)), (wg_hbm, wg_v, cols(0, 2 * T))],
        [(wg_hbm, wg_v, cols(2 * T, 2 * T))],
        [(x_hbm, x_v, rows(2 * T, 2 * T)), (gw_hbm, gw_v, whole)],
        [(wu_hbm, wu_v, cols(0, D))],
        [(x_hbm, x_v, rows(D, D))],
        [(x_hbm, x_v, rows(2 * D, 2 * D)), (wg_hbm, wg_v, cols(D, D))],
        [(wu_hbm, wu_v, cols(D, D)), (wqkv_hbm, wqkv_v, cols(D, D))],
        [(wqkv_hbm, wqkv_v, cols(0, D)), (wg_hbm, wg_v, cols(2 * D, F - 2 * D)),
         (wu_hbm, wu_v, cols(2 * D, F - 2 * D))],
        [(wqkv_hbm, wqkv_v, cols(2 * D, D)), (wo_hbm, wo_v, whole), (wd_hbm, wd_v, rows(0, FT))],
        [(wd_hbm, wd_v, rows(FT, F - FT))],
    ])]

    def ffn(kind, u, s, result, then=None, left=3, **kw):
        def hook():
            for r in range(4):
                for n in range(4):
                    if r >= 2 or (n if kind == "gate" else 3 - n) >= 2:
                        result(u, s, r, n)
            wait(then)
        project((kind, u), s, left=left if then else 0, hook=hook, **kw)
        every_tile(result, u, s)

    wait(loads[0])
    first_gate(0, {0: 0, 1: 0})
    wait(loads[1])
    ws["gate", 0] = prepare(RHS, gate_tile(0), 1, (3, 2, 0, 5))
    first_gate(0, {2: 0.59, 3: 0.41})
    wait(loads[2])
    prepare_x(0, 1)
    first_gate(2, {0: 0.27, 1: 0.27, 2: 0.27, 3: 0.19})
    wait(loads[3])
    prepare_up(0, 0)
    ffn("up", 0, 0, hidden, loads[4], left=1)
    ws["gate", 0].update(prepare(RHS, gate_tile(0), 0, (1, 4, 6)))
    for s in range(1, NS):
        prepare_x(s, 0)
        project(("up", 0), s, amount=0)
        if s == 2:
            prepare_gate(1, 2)
        ffn("gate", 0, s, hidden, {1: loads[5], 3: loads[6]}.get(s))

    prepare_k(2.4)
    prepare_up(1, 1.6)
    for s in range(NS):
        ffn("gate", 1, s, act, {3: loads[7]}.get(s))

    cost = 8 / 4.5
    prepare_q(1.5 * cost)
    prepare_tail(cost)
    prepare_gate(2, cost)
    prepare_up(2, cost)
    for s in range(NS):
        strassen2(("k", s), lambda p, q: _nt(ws["k"][p, q], xs[s][p, q]))
        every_tile(phi_kt, s)
    for s in range(NS):
        ffn("up", 1, s, hidden, {3: loads[8]}.get(s))

    down = [prepare(RHS, lambda c, n, u=u: load(wd_v, u * D + c * T, n * T), 4.5)
            for u in range(3)]
    down.append(prepare(
        RHS, lambda t, n: regroup([v[:, n * T:(n + 1) * T] for v in kv_wo()], t), 4.5))
    strassen2("ktx", lambda p, q: _sum4(
        [_nn(ks[s](p, q).astype(bf16), xs[s][RHS_AS_LHS[p], RHS_AS_LHS[q]]) for s in range(NS)]),
        amount=6, pace=dict.fromkeys(OUTER_ORDER, 1))
    project("tail", 0)
    kv()
    project("tail", 1)
    kv_wo()
    project("tail", 2)
    project("tail", 3)
    for s in range(NS):
        project("q", s, amount=0)
        for r in range(4):
            attention(s, r)
            hidden_tail(s, r, 0)
            hidden_tail(s, r, 1)
    for s in range(NS):
        ffn("gate", 2, s, act)
    for s in range(NS):
        ffn("up", 2, s, hidden, {3: loads[9]}.get(s))

    for s in range(NS):
        output(s, down)
    wait(stores)


@jax.jit
def pallas_gated_mix__linear_attn_block__swiglu_ffn__prompt_kernel(
    A_x: jax.Array,
    A_wqkv: jax.Array,
    A_wo: jax.Array,
    B_x: jax.Array,
    B_w_gate: jax.Array,
    B_w_up: jax.Array,
    B_w_down: jax.Array,
    gate_w: jax.Array,
):
    del B_x
    assert A_x.shape == (1, S, D) and B_w_gate.shape == (D, F)
    inputs = (A_x.reshape(S, D), A_wqkv, A_wo, B_w_gate, B_w_up, B_w_down, gate_w)
    in_hbm = pl.BlockSpec(memory_space=pl.ANY)
    out = pl.pallas_call(
        _kernel,
        in_specs=[in_hbm] * len(inputs),
        out_specs=in_hbm,
        out_shape=jax.ShapeDtypeStruct((S, D), bf16),
        scratch_shapes=[pltpu.VMEM(v.shape, bf16) for v in inputs]
        + [pltpu.VMEM((S, D), bf16), pltpu.SemaphoreType.DMA((11,))],
        compiler_params=pltpu.CompilerParams(
            vmem_limit_bytes=120 * 2**20, disable_semaphore_checks=True),
        name="gated_mix",
    )(*inputs)
    return out.reshape(1, S, D)
```

```python
import functools

import jax
import jax.numpy as jnp
from jax import lax
import jax.experimental.pallas as pl
import jax.experimental.pallas.tpu as pltpu

S, D, F, DH = 2048, 512, 1792, 16
T = 128
NS = S // D
FT = 3 * D
STRIP = 16
f32, bf16, u32 = jnp.float32, jnp.bfloat16, jnp.uint32
lazy = functools.cache

LHS = [((0, 1), (3, 1)), ((2, 1), (3, 1)), ((0, 1),), ((3, 1),),
       ((0, 1), (1, 1)), ((2, 1), (0, -1)), ((1, 1), (3, -1))]
RHS = [((0, 1), (3, 1)), ((0, 1),), ((1, 1), (3, -1)), ((2, 1), (0, -1)),
       ((3, 1),), ((0, 1), (1, 1)), ((2, 1), (3, 1))]
OUT = [((0, 1), (3, 1), (4, -1), (6, 1)), ((2, 1), (4, 1)),
       ((1, 1), (3, 1)), ((0, 1), (1, -1), (2, 1), (5, 1))]
RHS_AS_LHS = [LHS.index(terms) for terms in RHS]
OUTER_ORDER = (1, 3, 2, 4, 0, 5, 6)
INNER_ORDER = (4, 2, 3, 6, 0, 1, 5)
PACE = dict(zip(OUTER_ORDER, (1, 0.25, 1, 0.25, 1, 0.25, 0)))


def _nn(a, b):
    return jnp.dot(a, b, preferred_element_type=f32)


def _nt(a, b):
    return lax.dot_general(a, b, (((1,), (1,)), ((), ())), preferred_element_type=f32)


def _signed_sum(terms):
    if terms[0][1] < 0:
        terms = [terms[1], terms[0], *terms[2:]]
    total = terms[0][0]
    for v, sign in terms[1:]:
        total = total + v if sign > 0 else total - v
    return total


def _sum4(v):
    return (v[0] + v[1]) + (v[2] + v[3])


def _tile(outer, inner):
    return 2 * (outer // 2) + inner // 2, 2 * (outer % 2) + inner % 2


def _combine(product, quadrant, order, init=None):
    terms = sorted(OUT[quadrant], key=lambda t: order.index(t[0]))
    terms = [(product(i), sign) for i, sign in terms]
    return _signed_sum(terms if init is None else [(init, 1)] + terms)


def _operands1(spec, tile):
    tile = lazy(tile)
    return lazy(lambda q: _signed_sum(
        [(tile(b // 2, b % 2), sign) for b, sign in spec[q]]).astype(bf16))


def _left_operands2(tile):
    tile = lazy(tile)

    @lazy
    def operand(p, q):
        t = [(tile(*_tile(a, b)), sa * sb) for a, sa in LHS[p] for b, sb in LHS[q]]
        return _signed_sum([t[0], t[3], t[1], t[2]] if len(t) == 4 else t)
    return operand


def _phi(t):
    return (jnp.maximum(t, 0.0) + 1e-6) + jnp.exp(jnp.minimum(t, 0.0))


def _silu_of_double(h):
    return h * jnp.tanh(h) + h


def _kernel(x_hbm, wqkv_hbm, wo_hbm, wg_hbm, wu_hbm, wd_hbm, gw_hbm, o_hbm,
            x_v, wqkv_v, wo_v, wg_v, wu_v, wd_v, gw_v, o_v, sems):

    def start(sem, *items):
        copies = [pltpu.make_async_copy(view(src), view(dst), sems.at[sem])
                  for src, dst, view in items]
        for c in copies:
            c.start()
        return copies

    def wait(copies):
        assert not queue
        for c in copies:
            c.wait()

    def cols(c0, n):
        return lambda ref: ref.at[:, pl.ds(c0, n)]

    def rows(r0, n):
        return lambda ref: ref.at[pl.ds(r0, n)]

    def whole(ref):
        return ref

    def load(ref, r0, c0):
        return ref[pl.ds(r0, T), pl.ds(c0, T)].astype(f32)

    lane = lazy(lambda n: lax.broadcasted_iota(jnp.int32, (n, T), 1))

    queue, state = [], {"credit": 0.0, "count": 0}
    never = lazy(lambda n: (lane(n) * (lane(n) + 1)) & 1 == 1)

    def advance(amount, result):
        state["credit"] += amount
        state["count"] += 1
        due = []
        while queue and state["credit"] >= queue[0][1] - 1e-6:
            step, cost = queue.pop(0)
            state["credit"] -= cost
            due.append(step)
        if not queue:
            state["credit"] = 0.0
        strips = result.shape[0] // STRIP
        shift = 3 * state["count"] if result.shape[0] == T else 0
        for i, step in enumerate(due):
            def after(v, r0=(i * strips // len(due) + shift) % strips * STRIP):
                n = v.shape[0]
                other = result[r0:r0 + n] if n == STRIP else result[:n]
                return jnp.where(never(n), lax.bitcast_convert_type(other, v.dtype), v)
            step(after)
        return result

    def prepare(spec, tile, cost, outer=range(7)):
        tile, parts, operands = lazy(tile), {}, {}

        def step(r0, p, after):
            t = [_signed_sum([(tile(*_tile(a, b))[r0:r0 + STRIP], sign) for a, sign in spec[p]])
                 for b in range(4)]
            t[0], t[3] = after(t[0]), after(t[3])
            for q in range(7):
                parts.setdefault((p, q), []).append(
                    _signed_sum([(t[b], sign) for b, sign in spec[q]]))
                if r0 + STRIP == T:
                    operands[p, q] = jnp.concatenate(parts[p, q]).astype(bf16)

        for r0 in range(0, T, STRIP):
            for p in outer:
                if cost:
                    queue.append(
                        (functools.partial(step, r0, p), cost * STRIP / (len(outer) * T)))
                else:
                    step(r0, p, lambda v: v)
        return operands

    def strassen1(product, amount=0):
        results = {q: advance(amount, product(q)) for q in INNER_ORDER}
        return [_combine(results.get, k, INNER_ORDER) for k in range(4)]

    mm = {}

    def strassen2(name, product, amount=1, pace=PACE, left=0, hook=None):
        m, remaining = {}, [49]
        mm[name] = lazy(lambda r, n: _combine(
            lambda p: m[p][2 * (r % 2) + n % 2], 2 * (r // 2) + n // 2, OUTER_ORDER))

        def issue(p, q):
            if remaining[0] == left:
                hook()
            remaining[0] -= 1
            return product(p, q)

        for p in OUTER_ORDER:
            m[p] = strassen1(functools.partial(issue, p),
                             amount * pace[p] / (7 * sum(pace.values())))

    xs, ws = {}, {}

    def project(w, s, **kw):
        strassen2((w, s), lambda p, q: _nn(xs[s][p, q], ws[w][p, q]), **kw)

    def every_tile(f, *args):
        for r in range(4):
            for n in range(4):
                f(*args, r, n)

    x_tile = lazy(lambda s, r, c: load(x_v, s * D + r * T, c * T))

    @lazy
    def ffn_gate(s, r):
        gw = gw_v[...].astype(f32).reshape(1, D)
        t = _sum4([x_tile(s, r, c) * gw[:, c * T:(c + 1) * T] for c in range(4)])
        t = jnp.sum(t, axis=-1, keepdims=True)
        return jnp.broadcast_to(0.5 - 0.5 * jnp.tanh(0.5 * t), (T, T))

    def prepare_x(s, cost):
        xs[s] = prepare(LHS, functools.partial(x_tile, s), cost)
        for r in range(4):
            ffn_gate(s, r)

    def gate_tile(u):
        return lambda c, n: 0.5 * load(wg_v, c * T, u * D + n * T)

    def prepare_gate(u, cost):
        ws["gate", u] = prepare(RHS, gate_tile(u), cost)

    def prepare_up(u, cost):
        ws["up", u] = prepare(RHS, lambda c, n: load(wu_v, c * T, u * D + (3 - n) * T), cost)

    act = lazy(lambda u, s, r, n: _silu_of_double(mm[("gate", u), s](r, n)))
    hidden = lazy(lambda u, s, r, n:
                  (act(u, s, r, n) * mm[("up", u), s](r, 3 - n)) * ffn_gate(s, r))

    first = {}
    mm[("gate", 0), 0] = lambda r, n: first[r, n]

    def first_gate(r0, shares):
        for n, amount in shares.items():
            v = advance(amount, _nn(x_v[pl.ds(r0 * T, 2 * T), :], wg_v[:, pl.ds(n * T, T)]))
            for i in range(2):
                first[r0 + i, n] = 0.5 * v[i * T:(i + 1) * T]
                act(0, 0, r0 + i, n)

    low = lazy(lambda: lane(T) < T // 2)

    def prepare_tail(cost):
        def tile(c, n):
            g = 0.5 * load(wg_v, c * T, FT + (n // 2) * T)
            v = load(wu_v, c * T, FT + (n // 2) * T)
            if n % 2:
                return pltpu.roll(jnp.where(low(), v, g), T // 2, 1)
            return jnp.where(low(), g, v)
        ws["tail"] = prepare(RHS, tile, cost)

    @lazy
    def hidden_tail(s, r, j):
        a = mm["tail", s](r, 2 * j)
        b = pltpu.roll(mm["tail", s](r, 2 * j + 1), T // 2, 1)
        return (_silu_of_double(jnp.where(low(), a, b)) * jnp.where(low(), b, a)) * ffn_gate(s, r)

    def by_dim(r0, n, c0, after):
        words = after(pltpu.bitcast(wqkv_v[pl.ds(r0, n), pl.ds(c0, T)], u32))
        return jnp.take_along_axis(words, (lane(n // 2) % 8) * DH + lane(n // 2) // 8, axis=1)

    def regroup(tiles, t):
        return jnp.concatenate([v[8 * d:8 * d + 8] for d in range(4 * t, 4 * t + 4) for v in tiles])

    def prepare_k(cost):
        wt = {}

        def transpose(c, n, after):
            wt[c, n] = pltpu.bitcast(by_dim(c * T, T, D + n * T, after), bf16).astype(f32).T
        queue.extend((functools.partial(transpose, c, n), cost / 48)
                     for c in range(4) for n in range(4))
        ws["k"] = prepare(RHS, lambda c, n: wt[c, n], cost * 2 / 3)

    def prepare_q(cost):
        wt, w = {}, {}

        def there(c, n, after):
            wt[c, n] = by_dim(2 * c * T, 2 * T, n * T, after).T

        def back(c, t, after):
            w[c, t] = pltpu.bitcast(after(regroup([wt[c, n] for n in range(4)], t)).T, bf16)
        queue.extend((functools.partial(f, c, n), cost / 48)
                     for f in (there, back) for c in range(2) for n in range(4))
        ws["q"] = prepare(
            RHS, lambda c, t: w[c // 2, t][(c % 2) * T:(c % 2 + 1) * T].astype(f32), cost * 2 / 3)

    phi_kt = lazy(lambda s, n, r: _phi(mm["k", s](r, n)))
    ks = [_left_operands2(functools.partial(phi_kt, s)) for s in range(NS)]

    @lazy
    def kv():
        same_head = lax.broadcasted_iota(jnp.int32, (T, T), 0) % 8 == lane(T) // DH
        out = []
        for n in range(4):
            ktx = jnp.concatenate([mm["ktx"](n, c) for c in range(4)], axis=1).astype(bf16)
            v = _nn(ktx, wqkv_v[:, pl.ds(2 * D + n * T, T)])
            out.append(jnp.where(same_head, v, 0.0).astype(bf16))
        return out

    kv_wo = lazy(lambda: [_nn(kv()[n], wo_v[pl.ds(n * T, T), :]) for n in range(4)])

    @lazy
    def z():
        sums = [_sum4([ks[s]((4, 1)[n // 2], (4, 1)[n % 2]) for s in range(NS)])
                for n in range(4)]
        return [jnp.sum(regroup(sums, t).T, axis=0, keepdims=True) for t in range(4)]

    @lazy
    def attention(s, r):
        phi_q = [_phi(mm["q", s](r, t)) for t in range(4)]
        den = _sum4([phi_q[t] * z()[t] for t in range(4)])
        den = den + pltpu.roll(den, 64, 1)
        den = den + pltpu.roll(den, 32, 1)
        return phi_q, (1.0 - ffn_gate(s, r)) * pltpu.reciprocal(den + 1e-6, full_range=False)

    stores = []
    down_tail = [_operands1(RHS, lambda i, j, n=n: load(wd_v, FT + i * T, (2 * n + j) * T))
                 for n in range(2)]

    def output(s, down):
        def store(r0, c0, n):
            view = lambda ref: ref.at[pl.ds(s * D + r0 * T, n * T), pl.ds(c0 * T, n * T)]
            stores.extend(start(4, (o_v, o_hbm, view)))

        hs = [_left_operands2(functools.partial(hidden, u, s)) for u in range(3)]
        hs.append(_left_operands2(lambda r, t: attention(s, r)[0][t] * attention(s, r)[1]))
        ht = [_operands1(LHS, lambda i, j, h=h: hidden_tail(s, 2 * h + i, j)) for h in range(2)]
        tail = [strassen1(lambda q: _nn(ht[k // 2](q), down_tail[k % 2](q))) for k in range(4)]
        m = {}
        for p in OUTER_ORDER:
            m[p] = strassen1(lambda q: _sum4(
                [_nn(hs[u](p, q).astype(bf16), down[u][p, q]) for u in range(4)]))
            for outer in range(4):
                needs = dict(OUT[outer])
                if p not in needs or any(i not in m for i in needs):
                    continue
                for inner in (1, 0, 2, 3):
                    r, n = _tile(outer, inner)
                    v = _combine(lambda i: m[i][inner], outer, OUTER_ORDER, tail[outer][inner])
                    o_v[pl.ds(s * D + r * T, T), pl.ds(n * T, T)] = v.astype(bf16)
                    if s == NS - 1 and len(m) == 7:
                        store(r, n, 1)
                if s == NS - 1 and len(m) < 7:
                    store(*_tile(outer, 0), 2)
        if s < NS - 1:
            store(0, 0, 4)

    loads = [start(i, *items) for i, items in enumerate([
        [(x_hbm, x_v, rows(0, 2 * T)), (wg_hbm, wg_v, cols(0, 2 * T))],
        [(wg_hbm, wg_v, cols(2 * T, 2 * T))],
        [(x_hbm, x_v, rows(2 * T, 2 * T)), (gw_hbm, gw_v, whole)],
        [(wu_hbm, wu_v, cols(0, D))],
        [(x_hbm, x_v, rows(D, D))],
        [(x_hbm, x_v, rows(2 * D, 2 * D)), (wg_hbm, wg_v, cols(D, D))],
    ])]
    later_loads = [
        [(wu_hbm, wu_v, cols(D, D)), (wqkv_hbm, wqkv_v, cols(D, D))],
        [(wqkv_hbm, wqkv_v, cols(0, D)), (wg_hbm, wg_v, cols(2 * D, F - 2 * D)),
         (wu_hbm, wu_v, cols(2 * D, F - 2 * D))],
        [(wqkv_hbm, wqkv_v, cols(2 * D, D)), (wo_hbm, wo_v, whole), (wd_hbm, wd_v, rows(0, FT))],
        [(wd_hbm, wd_v, rows(FT, F - FT))],
    ]

    def ffn(kind, u, s, result, then=None, left=3, **kw):
        def hook():
            for r in range(4):
                for n in range(4):
                    if r >= 2 or (n if kind == "gate" else 3 - n) >= 2:
                        result(u, s, r, n)
            wait(then)
        project((kind, u), s, left=left if then else 0, hook=hook, **kw)
        every_tile(result, u, s)

    wait(loads[0])
    first_gate(0, {0: 0, 1: 0})
    wait(loads[1])
    ws["gate", 0] = prepare(RHS, gate_tile(0), 1, (3, 2, 0, 5))
    first_gate(0, {2: 0.59, 3: 0.41})
    wait(loads[2])
    prepare_x(0, 1)
    first_gate(2, {0: 0.27, 1: 0.27, 2: 0.27, 3: 0.19})
    wait(loads[3])
    loads += [start(i, *items) for i, items in enumerate(later_loads)]
    prepare_up(0, 0)
    ffn("up", 0, 0, hidden, loads[4], left=1)
    ws["gate", 0].update(prepare(RHS, gate_tile(0), 0, (1, 4, 6)))
    for s in range(1, NS):
        prepare_x(s, 0)
        project(("up", 0), s, amount=0)
        if s == 2:
            prepare_gate(1, 2)
        ffn("gate", 0, s, hidden, {1: loads[5], 3: loads[6]}.get(s))

    prepare_k(2.4)
    prepare_up(1, 1.6)
    for s in range(NS):
        ffn("gate", 1, s, act, {3: loads[7]}.get(s))

    cost = 8 / 4.5
    prepare_q(1.5 * cost)
    prepare_tail(cost)
    prepare_gate(2, cost)
    prepare_up(2, cost)
    for s in range(NS):
        strassen2(("k", s), lambda p, q: _nt(ws["k"][p, q], xs[s][p, q]))
        every_tile(phi_kt, s)
    for s in range(NS):
        ffn("up", 1, s, hidden, {3: loads[8]}.get(s))

    down = [prepare(RHS, lambda c, n, u=u: load(wd_v, u * D + c * T, n * T), 4.5)
            for u in range(3)]
    down.append(prepare(
        RHS, lambda t, n: regroup([v[:, n * T:(n + 1) * T] for v in kv_wo()], t), 4.5))
    strassen2("ktx", lambda p, q: _sum4(
        [_nn(ks[s](p, q).astype(bf16), xs[s][RHS_AS_LHS[p], RHS_AS_LHS[q]]) for s in range(NS)]),
        amount=6, pace=dict.fromkeys(OUTER_ORDER, 1))
    project("tail", 0)
    kv()
    project("tail", 1)
    kv_wo()
    project("tail", 2)
    project("tail", 3)
    for s in range(NS):
        project("q", s, amount=0)
        for r in range(4):
            attention(s, r)
            hidden_tail(s, r, 0)
            hidden_tail(s, r, 1)
    for s in range(NS):
        ffn("gate", 2, s, act)
    for s in range(NS):
        ffn("up", 2, s, hidden, {3: loads[9]}.get(s))

    for s in range(NS):
        output(s, down)
    wait(stores)


@jax.jit
def pallas_gated_mix__linear_attn_block__swiglu_ffn__prompt_kernel(
    A_x: jax.Array,
    A_wqkv: jax.Array,
    A_wo: jax.Array,
    B_x: jax.Array,
    B_w_gate: jax.Array,
    B_w_up: jax.Array,
    B_w_down: jax.Array,
    gate_w: jax.Array,
):
    del B_x
    assert A_x.shape == (1, S, D) and B_w_gate.shape == (D, F)
    inputs = (A_x.reshape(S, D), A_wqkv, A_wo, B_w_gate, B_w_up, B_w_down, gate_w)
    in_hbm = pl.BlockSpec(memory_space=pl.ANY)
    out = pl.pallas_call(
        _kernel,
        in_specs=[in_hbm] * len(inputs),
        out_specs=in_hbm,
        out_shape=jax.ShapeDtypeStruct((S, D), bf16),
        scratch_shapes=[pltpu.VMEM(v.shape, bf16) for v in inputs]
        + [pltpu.VMEM((S, D), bf16), pltpu.SemaphoreType.DMA((6,))],
        compiler_params=pltpu.CompilerParams(vmem_limit_bytes=120 * 2**20),
        name="gated_mix",
    )(*inputs)
    return out.reshape(1, S, D)
```
